```python
import jax
import jax.numpy as jnp

def _softmax(x, axis=-1):
    return jax.nn.softmax(x, axis=axis)

def _gelu(x):
    return jax.nn.gelu(x, approximate=True)

def _silu(x):
    return jax.nn.silu(x)

def _sigmoid(x):
    return jax.nn.sigmoid(x)

def _layernorm(x, axis=-1, eps=1e-05):
    m = jnp.mean(x, axis=axis, keepdims=True)
    v = jnp.var(x, axis=axis, keepdims=True)
    return (x - m) / jnp.sqrt(v + eps)

def _scatter_add(tgt, idx, src, axis=0):
    return tgt.at[idx].add(src)

def _segment_sum(src, seg, n):
    return jax.ops.segment_sum(src, seg, n)

class _Rng:

    def __init__(self, key):
        self._k = key

    def _next(self):
        self._k, sub = jax.random.split(self._k)
        return sub

    def normal(self, shape):
        return jax.random.normal(self._next(), shape, dtype=jnp.bfloat16)

    def randint(self, lo, hi, shape):
        return jax.random.randint(self._next(), shape, lo, hi, dtype=jnp.int32)

    def uniform(self, shape, lo=0.0, hi=1.0):
        return jax.random.uniform(self._next(), shape, jnp.bfloat16, lo, hi)

    def permutation(self, n):
        return jax.random.permutation(self._next(), n)
kernel_name = 'adaLN_cond__sliding_block_cached__dense_activation_mish__decode'

def setup_inputs():
    _rng = _Rng(jax.random.key(int.from_bytes(__import__("os").urandom(4), "little")))
    _w = lambda a: (lambda t: t.astype(jnp.bfloat16) if jnp.issubdtype(t.dtype, jnp.floating) else t)(jnp.asarray(a))

    def _A_setup():
        B, Sq, D = (1, 1, 640)
        Hq, Hkv, Sk, Dh = (32, 32, 32768, 192)
        assert Hq % Hkv == 0, (Hq, Hkv)
        return {'x': _w((lambda *s: _rng.normal(s) * 0.05)(B, Sq, D)), 'k_cache': _w((lambda *s: _rng.normal(s) * 0.05)(B, Hkv, Sk, Dh)), 'v_cache': _w((lambda *s: _rng.normal(s) * 0.05)(B, Hkv, Sk, Dh)), 'wq': _w((lambda *s: _rng.normal(s) * 0.05)(D, Hq * Dh) * D ** (-0.5)), 'wo': _w((lambda *s: _rng.normal(s) * 0.05)(Hq * Dh, D) * (Hq * Dh) ** (-0.5))}
    _A_in = _A_setup()

    def _B_setup():
        B, S, D, F = (1, 1, 640, 1536)
        return {'x': _w((lambda *s: _rng.normal(s) * 0.05)(B, S, D)), 'w1': _w((lambda *s: _rng.normal(s) * 0.05)(D, F) * D ** (-0.5)), 'b1': _w((lambda *s: _rng.normal(s) * 0.05)(F)), 'w2': _w((lambda *s: _rng.normal(s) * 0.05)(F, D) * F ** (-0.5))}
    _B_in = _B_setup()
    return {'A_x': _A_in['x'], 'A_k_cache': _A_in['k_cache'], 'A_v_cache': _A_in['v_cache'], 'A_wq': _A_in['wq'], 'A_wo': _A_in['wo'], 'B_x': _B_in['x'], 'B_w1': _B_in['w1'], 'B_b1': _B_in['b1'], 'B_w2': _B_in['w2'], 'c': _w((lambda *s: _rng.normal(s) * 0.05)(1, 640)), 'w_mod': _w((lambda *s: _rng.normal(s) * 0.05)(640, 6 * 640) * 640 ** (-0.5))}

def reference(A_x, A_k_cache, A_v_cache, A_wq, A_wo, B_x, B_w1, B_b1, B_w2, c, w_mod):

    def _A_ref(x, k_cache, v_cache, wq, wo):
        B, Sq, D = x.shape
        Hq, Dh = (32, 192)
        Hkv, Sk = (k_cache.shape[1], k_cache.shape[2])
        W = min(4096, max(256, Sk // 4))
        rep = Hq // Hkv
        q = (lambda x, *d: x.transpose(*d))((x @ wq).reshape(B, Sq, Hq, Dh), 0, 2, 1, 3)
        k = jnp.repeat(k_cache[:, :, Sk - W:, :], rep, axis=1)
        v = jnp.repeat(v_cache[:, :, Sk - W:, :], rep, axis=1)
        scores = jnp.einsum('bhqd,bhkd->bhqk', q, k) * Dh ** (-0.5)
        p = _softmax(scores, axis=-1)
        o = jnp.einsum('bhqk,bhkd->bhqd', p, v)
        return (lambda x, *d: x.transpose(*d))(o, 0, 2, 1, 3).reshape(B, Sq, Hq * Dh) @ wo

    def _B_ref(x, w1, b1, w2):
        h = jnp.einsum('bsd,df->bsf', x, w1) + b1
        sp = jnp.log1p(jnp.exp(-jnp.abs(h))) + jnp.where(h > 0, h, jnp.zeros_like(h))
        act = h * jnp.tanh(sp)
        return jnp.einsum('bsf,fd->bsd', act, w2)
    x = A_x
    mod = (_silu(c) @ w_mod).reshape(c.shape[0], 6, 1, -1)
    sa, ca, ga, sb, cb, gb = (mod[:, 0].copy(), mod[:, 1].copy(), mod[:, 2].copy(), mod[:, 3].copy(), mod[:, 4].copy(), mod[:, 5].copy())
    h = _layernorm(x, axis=-1) * (1 + ca) + sa
    x = x + ga * _A_ref(h, A_k_cache, A_v_cache, A_wq, A_wo)
    h = _layernorm(x, axis=-1) * (1 + cb) + sb
    x = x + gb * _B_ref(h, B_w1, B_b1, B_w2)
    return x
```

```python
import functools

import jax
import jax.numpy as jnp
from jax import lax
import jax.experimental.pallas as pl
import jax.experimental.pallas.tpu as pltpu

D = 640
H = 32
DH = 192
F = 1536
PAIR = 2 * DH
NPAIR = H // 2
LANE = 128
F32 = jnp.float32
BF16 = jnp.bfloat16

KV_ROWS = 96
NSLOT = 3
LOOK = 96
LOOP_LOOK = 128
PACE = 10
QK_STEPS = 4
PV_STEPS = 4
W2_PARTS = 3


def _layernorm(x, eps=1e-5):
    m = jnp.mean(x, axis=-1, keepdims=True)
    d = x - m
    v = jnp.mean(d * d, axis=-1, keepdims=True)
    return d / jnp.sqrt(v + eps)


def _zip2(a, b):
    n = min(len(a), len(b))
    out = [x for p in zip(a[:n], b[:n]) for x in p]
    rest = a[n:] + b[n:]
    h = len(rest) // 2
    return out + [x for p in zip(rest[:h], rest[h:2 * h]) for x in p] + rest[2 * h:]


def _halves(a):
    return _zip2(a[:len(a) // 2], a[len(a) // 2:])


class _Stream:
    def __init__(self, parts, fence=None):
        self.copies = [cp for part in parts for cp in part]
        self.bounds = set()
        n = 0
        for part in parts[:-1]:
            n += len(part)
            self.bounds.add(n)
        self.fence = fence
        self.pos = 0

    def upto(self, n):
        n = min(n, len(self.copies))
        while self.pos < n:
            if self.fence is not None and self.pos in self.bounds:
                self.fence()
            self.copies[self.pos]().start(priority=self.pos % 2)
            self.pos += 1

    def more(self, k):
        self.upto(self.pos + k)

    def rest(self):
        self.upto(len(self.copies))


def _weight_copies(src, dst, sem, shape, rows_first, jump, rows=None, cols=None):
    r0, r1 = rows or (0, src.shape[0])
    c0, c1 = cols or (0, src.shape[1])
    rr, cc = shape
    if rows_first:
        idx = [(r, c) for c in range(c0, c1, cc) for r in range(r0, r1, rr)]
    else:
        idx = [(r, c) for r in range(r0, r1, rr) for c in range(c0, c1, cc)]
    idx = [idx[i] for o in range(jump) for i in range(o, len(idx), jump)]
    return [functools.partial(pltpu.make_async_copy, src.at[pl.ds(r, rr), pl.ds(c, cc)],
                              dst.at[pl.ds(r, rr), pl.ds(c, cc)], sem) for r, c in idx]


def _wait_all(buf, sem):
    pltpu.make_async_copy(buf, buf, sem).wait()


def _kernel(x_hbm, k_hbm, v_hbm, wq_hbm, wo_hbm, w1_hbm, b1_hbm, w2_hbm, c_hbm, wmod_hbm, o_ref,
            x_v, c_v, b1_v, wmod_v, wq_v, wo_v, w1_v, w2_v, kbuf, vbuf, q_s, s_s, att_s,
            sem_w, sem_kv, sem_f, *, window):
    sk = k_hbm.shape[1]
    nc = window // LANE

    def kv_copies(p, slot):
        out = []
        for r in range(0, PAIR, KV_ROWS):
            row = p * PAIR + r
            if not isinstance(row, int):
                row = pl.multiple_of(row, 8)
            for c in range(nc):
                for j, (src, dst) in enumerate(((k_hbm, kbuf), (v_hbm, vbuf))):
                    out.append(functools.partial(
                        pltpu.make_async_copy,
                        src.at[pl.ds(row, KV_ROWS), pl.ds(sk - window + c * LANE, LANE)],
                        dst.at[slot, c, pl.ds(r, KV_ROWS), :], sem_kv.at[j, slot]))
        return out

    def fence():
        pl.semaphore_wait(sem_f, 0)

    s_c, s_x, s_b1, s_wa, s_wb, s_wq, s_wo, s_w1, s_w2 = range(9)
    small = [functools.partial(pltpu.make_async_copy, s, d, sem_w.at[i])
             for i, s, d in ((s_c, c_hbm, c_v), (s_x, x_hbm, x_v), (s_b1, b1_hbm, b1_v))]
    l_wa = _halves(_weight_copies(wmod_hbm, wmod_v, sem_w.at[s_wa], (16, 640), True, 4, cols=(0, 2 * D)))
    l_wb = _halves(_weight_copies(wmod_hbm, wmod_v, sem_w.at[s_wb], (16, 640), True, 4, cols=(2 * D, 6 * D)))
    l_wq = _weight_copies(wq_hbm, wq_v, sem_w.at[s_wq], (16, 1024), True, 8)
    l_wo = _weight_copies(wo_hbm, wo_v, sem_w.at[s_wo], (16, 640), False, 48)
    l_w1 = _halves(_weight_copies(w1_hbm, w1_v, sem_w.at[s_w1], (16, 768), True, 10))
    hr = F // 2 // W2_PARTS
    w2_rows = [((i * hr, (i + 1) * hr), (F // 2 + i * hr, F // 2 + (i + 1) * hr)) for i in range(W2_PARTS)]
    l_w2 = []
    for i, (ra, rb) in enumerate(w2_rows):
        l_w2 += _zip2(_weight_copies(w2_hbm, w2_v, sem_w.at[s_w2 + 2 * i], (16, 640), False, 1, rows=ra),
                      _weight_copies(w2_hbm, w2_v, sem_w.at[s_w2 + 2 * i + 1], (16, 640), False, 1, rows=rb))

    l_qo = _zip2(l_wq, l_wo)
    head = _Stream([l_wa, l_qo, kv_copies(0, 0), kv_copies(1, 1)[:LOOP_LOOK]], fence)
    head.more(2)
    for cp in small:
        cp().start()
    head.upto(len(l_wa) + LOOK)
    for cp in small:
        cp().wait()
    _wait_all(wmod_v.at[:, pl.ds(0, 2 * D)], sem_w.at[s_wa])
    cf = c_v[...].astype(F32)
    silu_c = jnp.broadcast_to(cf * jax.nn.sigmoid(cf), (8, D)).astype(BF16)

    def mod(i):
        return jnp.dot(silu_c, wmod_v[:, i * D:(i + 1) * D], preferred_element_type=F32)

    sa = mod(0)
    head.more(PACE)
    ca = mod(1)
    head.more(PACE)
    x0 = jnp.broadcast_to(x_v[...].astype(F32), (8, D))
    h = (_layernorm(x0) * (1.0 + ca) + sa).astype(BF16)
    head.upto(len(l_wa) + 2 * len(l_wq) + LOOK)
    _wait_all(wq_v, sem_w.at[s_wq])
    row = lax.broadcasted_iota(jnp.int32, (8, PAIR), 0)
    col = lax.broadcasted_iota(jnp.int32, (8, PAIR), 1)
    own = jnp.logical_or(jnp.logical_and(row == 0, col < DH), jnp.logical_and(row == 1, col >= DH))
    for p in range(NPAIR):
        qp = jnp.dot(h, wq_v[:, p * PAIR:(p + 1) * PAIR], preferred_element_type=F32)
        q_s[p] = jnp.where(own, qp, 0.0)
        head.more(PACE)
    head.rest()
    _wait_all(wo_v, sem_w.at[s_wo])
    att_s[...] = jnp.zeros(att_s.shape, F32)

    scale = DH ** -0.5

    def pair_step(p, slot, stream, step):
        _wait_all(kbuf.at[slot], sem_kv.at[0, slot])
        q = q_s[p].astype(BF16)
        per = nc // QK_STEPS
        for i in range(QK_STEPS):
            for c in range(i * per, (i + 1) * per):
                s_s[:, c * LANE:(c + 1) * LANE] = jnp.dot(q, kbuf[slot, c], preferred_element_type=F32) * scale
            stream.more(step)
        s = s_s[...]
        e = jnp.exp(s - jnp.max(s, axis=-1, keepdims=True))
        denom = jnp.sum(e, axis=-1, keepdims=True)
        s_s[...] = e
        stream.more(step)
        _wait_all(vbuf.at[slot], sem_kv.at[1, slot])
        acc = jnp.zeros((8, PAIR), F32)
        per = nc // PV_STEPS
        for i in range(PV_STEPS):
            for c in range(i * per, (i + 1) * per):
                acc += lax.dot_general(s_s[:, c * LANE:(c + 1) * LANE].astype(BF16), vbuf[slot, c],
                                       (((1,), (1,)), ((), ())), preferred_element_type=F32)
            stream.more(step)
        o = jnp.where(own, acc / denom, 0.0).astype(BF16)
        r0 = p * PAIR
        if not isinstance(r0, int):
            r0 = pl.multiple_of(r0, PAIR)
        att_s[...] += jnp.dot(o, wo_v[pl.ds(r0, PAIR), :], preferred_element_type=F32)

    per_pair = 2 * nc * (PAIR // KV_ROWS)

    def body(p, carry):
        st = _Stream([kv_copies(p + 1, (p + 1) % NSLOT)[LOOP_LOOK:], kv_copies(p + 2, (p + 2) % NSLOT)[:LOOP_LOOK]])
        pair_step(p, p % NSLOT, st, per_pair // (QK_STEPS + PV_STEPS + 2) // 2 * 2)
        st.rest()
        return carry

    lax.fori_loop(0, NPAIR - 2, body, 0)

    last = kv_copies(NPAIR - 1, (NPAIR - 1) % NSLOT)[LOOP_LOOK:]
    tail = _Stream([last, l_wb, l_w1, l_w2], fence)
    pair_step(NPAIR - 2, (NPAIR - 2) % NSLOT, tail, PACE)
    tail.upto(len(last) + LOOK)
    pair_step(NPAIR - 1, (NPAIR - 1) % NSLOT, tail, PACE)

    tail.upto(len(last) + len(l_wb) + LOOK)
    _wait_all(wmod_v.at[:, pl.ds(2 * D, 4 * D)], sem_w.at[s_wb])
    ga = mod(2)
    tail.more(PACE)
    att = jnp.broadcast_to(jnp.sum(att_s[...], axis=0, keepdims=True), (8, D))
    x1 = x0 + ga * att
    sb = mod(3)
    tail.more(PACE)
    cb = mod(4)
    tail.more(PACE)
    h2 = (_layernorm(x1) * (1.0 + cb) + sb).astype(BF16)
    gb = mod(5)
    tail.more(PACE)
    tail.upto(len(last) + len(l_wb) + len(l_w1) + LOOK)
    _wait_all(w1_v, sem_w.at[s_w1])
    b1 = b1_v[...].astype(F32)
    acts = []
    for j in range(3):
        u = jnp.dot(h2, w1_v[:, j * 512:(j + 1) * 512], preferred_element_type=F32)
        u = u + jnp.concatenate([jnp.broadcast_to(b1[t:t + 1, :], (8, LANE)) for t in range(4 * j, 4 * j + 4)], axis=1)
        softplus = jnp.log1p(jnp.exp(-jnp.abs(u))) + jnp.where(u > 0, u, 0.0)
        acts.append((u * jnp.tanh(softplus)).astype(BF16))
        tail.more(PACE)
    act = jnp.concatenate(acts, axis=1)
    tail.rest()
    y = jnp.zeros((8, D), F32)
    for i, rr in enumerate(w2_rows):
        for t, (ra, rb) in enumerate(rr):
            _wait_all(w2_v.at[pl.ds(ra, rb - ra)], sem_w.at[s_w2 + 2 * i + t])
            y += jnp.dot(act[:, ra:rb], w2_v[ra:rb, :], preferred_element_type=F32)
    o_ref[...] = (x1 + gb * y)[0:1].astype(o_ref.dtype)


@jax.jit
def pallas_adaLN_cond__sliding_block_cached__dense_activation_mish__decode_kernel(
    A_x: jax.Array,
    A_k_cache: jax.Array,
    A_v_cache: jax.Array,
    A_wq: jax.Array,
    A_wo: jax.Array,
    B_x: jax.Array,
    B_w1: jax.Array,
    B_b1: jax.Array,
    B_w2: jax.Array,
    c: jax.Array,
    w_mod: jax.Array,
):
    del B_x
    sk = A_k_cache.shape[2]
    window = min(4096, max(256, sk // 4))
    kt = jnp.swapaxes(A_k_cache, 2, 3).reshape(H * DH, sk)
    vt = jnp.swapaxes(A_v_cache, 2, 3).reshape(H * DH, sk)
    hbm = pl.BlockSpec(memory_space=pltpu.HBM)
    out = pl.pallas_call(
        functools.partial(_kernel, window=window),
        out_shape=jax.ShapeDtypeStruct((1, D), A_x.dtype),
        in_specs=[hbm] * 10,
        out_specs=pl.BlockSpec(memory_space=pltpu.VMEM),
        scratch_shapes=[
            pltpu.VMEM((1, D), BF16),
            pltpu.VMEM((1, D), BF16),
            pltpu.VMEM((F // LANE, LANE), BF16),
            pltpu.VMEM((D, 6 * D), BF16),
            pltpu.VMEM((D, H * DH), BF16),
            pltpu.VMEM((H * DH, D), BF16),
            pltpu.VMEM((D, F), BF16),
            pltpu.VMEM((F, D), BF16),
            pltpu.VMEM((NSLOT, window // LANE, PAIR, LANE), BF16),
            pltpu.VMEM((NSLOT, window // LANE, PAIR, LANE), BF16),
            pltpu.VMEM((NPAIR, 8, PAIR), F32),
            pltpu.VMEM((8, window), F32),
            pltpu.VMEM((8, D), F32),
            pltpu.SemaphoreType.DMA((8 + 2 * W2_PARTS,)),
            pltpu.SemaphoreType.DMA((2, NSLOT)),
            pltpu.SemaphoreType.REGULAR,
        ],
        compiler_params=pltpu.CompilerParams(
            vmem_limit_bytes=64 * 2**20,
            disable_bounds_checks=True,
            disable_semaphore_checks=True,
        ),
        name="adaln_attn_mlp_decode",
    )(A_x.reshape(1, D), kt, vt, A_wq, A_wo, B_w1, B_b1.reshape(F // LANE, LANE), B_w2, c, w_mod)
    return out.reshape(A_x.shape)
```

```python
import functools

import jax
import jax.numpy as jnp
from jax import lax
import jax.experimental.pallas as pl
import jax.experimental.pallas.tpu as pltpu

D = 640
H = 32
DH = 192
F = 1536
PAIR = 2 * DH
NPAIR = H // 2
LANE = 128
F32 = jnp.float32
BF16 = jnp.bfloat16

KV_ROWS = 96
NSLOT = 3
LOOK = 80
LOOP_LOOK = 128
PACE = 10
QK_STEPS = 4
PV_STEPS = 4
W1_PARTS = 2
W2_ROWS = (384, 256, 128)
W2_ORDER = ((0, 0), (0, 1), (1, 0), (2, 0), (1, 1), (2, 1))


def _layernorm(x, eps=1e-5):
    m = jnp.mean(x, axis=-1, keepdims=True)
    d = x - m
    v = jnp.mean(d * d, axis=-1, keepdims=True)
    return d / jnp.sqrt(v + eps)


def _mish(u):
    softplus = jnp.log1p(jnp.exp(-jnp.abs(u))) + jnp.where(u > 0, u, 0.0)
    return u * jnp.tanh(softplus)


def _dot(a, b):
    return jnp.dot(a, b, preferred_element_type=F32)


def _zip2(a, b):
    n = min(len(a), len(b))
    out = [x for p in zip(a[:n], b[:n]) for x in p]
    rest = a[n:] + b[n:]
    h = len(rest) // 2
    return out + [x for p in zip(rest[:h], rest[h:2 * h]) for x in p] + rest[2 * h:]


class _Stream:
    def __init__(self, parts, fence=None):
        self.copies = [cp for part in parts for cp in part]
        self.ends = []
        n = 0
        for part in parts:
            n += len(part)
            self.ends.append(n)
        self.fence = fence
        self.pos = 0

    def upto(self, n):
        n = min(n, len(self.copies))
        while self.pos < n:
            if self.fence is not None and self.pos in self.ends:
                self.fence()
            self.copies[self.pos]().start(priority=self.pos % 2)
            self.pos += 1

    def more(self, k):
        if self.fence is not None and self.pos < len(self.copies):
            self.fence()
        self.upto(self.pos + k)

    def past(self, part):
        self.upto(self.ends[part] + LOOK)

    def rest(self):
        self.upto(len(self.copies))


def _copies(src, dst, sem, shape, jump, rows=None, cols=None):
    r0, r1 = rows or (0, src.shape[0])
    c0, c1 = cols or (0, src.shape[1])
    rr, cc = shape
    assert (r1 - r0) % rr == 0 and (c1 - c0) % cc == 0
    idx = [(r, c) for c in range(c0, c1, cc) for r in range(r0, r1, rr)]
    idx = [idx[i] for o in range(jump) for i in range(o, len(idx), jump)]
    return [functools.partial(pltpu.make_async_copy, src.at[pl.ds(r, rr), pl.ds(c, cc)],
                              dst.at[pl.ds(r, rr), pl.ds(c, cc)], sem) for r, c in idx]


def _copies2(src, dst, sem, shape, jump, rows=None, cols=None):
    r0, r1 = rows or (0, src.shape[0])
    mid = (r0 + r1) // 2
    return _zip2(_copies(src, dst, sem, shape, jump, (r0, mid), cols),
                 _copies(src, dst, sem, shape, jump, (mid, r1), cols))


def _wait_all(buf, sem):
    pltpu.make_async_copy(buf, buf, sem).wait()


def _kernel(x_hbm, k_hbm, v_hbm, wq_hbm, wo_hbm, w1_hbm, b1_hbm, w2_hbm, c_hbm, wmod_hbm, o_ref,
            x_v, c_v, b1_v, wmod_v, wq_v, wo_v, w1_v, w2_v, kbuf, vbuf, q_s, s_s, att_s, mod_s,
            sem_w, sem_kv, sem_fence, *, window):
    sk = k_hbm.shape[1]
    nc = window // LANE

    def kv_copies(p, slot):
        out = []
        for r in range(0, PAIR, KV_ROWS):
            row = p * PAIR + r
            if not isinstance(row, int):
                row = pl.multiple_of(row, 8)
            for c in range(nc):
                for j, (src, dst) in enumerate(((k_hbm, kbuf), (v_hbm, vbuf))):
                    out.append(functools.partial(
                        pltpu.make_async_copy,
                        src.at[pl.ds(row, KV_ROWS), pl.ds(sk - window + c * LANE, LANE)],
                        dst.at[slot, c, pl.ds(r, KV_ROWS), :], sem_kv.at[j, slot]))
        return out

    def fence():
        pl.semaphore_wait(sem_fence, 0)

    s_c, s_x, s_b1, s_wmod, s_wq, s_wo, s_wo_tail, s_w1 = range(8)
    s_w2 = s_w1 + W1_PARTS
    small = [functools.partial(pltpu.make_async_copy, s, d, sem_w.at[i])
             for i, s, d in ((s_c, c_hbm, c_v), (s_x, x_hbm, x_v), (s_b1, b1_hbm, b1_v))]
    wo_split = (NPAIR - 2) * PAIR

    head = _Stream([
        _copies2(wmod_hbm, wmod_v, sem_w.at[s_wmod], (8, 1280), 8),
        _zip2(_copies(wq_hbm, wq_v, sem_w.at[s_wq], (8, 1536), 8),
              _copies(wo_hbm, wo_v, sem_w.at[s_wo], (24, D), 48, rows=(0, wo_split))),
        kv_copies(0, 0),
        kv_copies(1, 1)[:LOOP_LOOK],
    ], fence)
    head.upto(2)
    for cp in small:
        cp().start()
    head.past(0)
    for cp in small:
        cp().wait()
    _wait_all(wmod_v, sem_w.at[s_wmod])
    cf = c_v[...].astype(F32)
    silu_c = jnp.broadcast_to(cf * jax.nn.sigmoid(cf), (8, D)).astype(BF16)
    for i in range(6):
        mod_s[i] = _dot(silu_c, wmod_v[:, i * D:(i + 1) * D])
        head.more(PACE)
    x0 = jnp.broadcast_to(x_v[...].astype(F32), (8, D))
    h = (_layernorm(x0) * (1.0 + mod_s[1]) + mod_s[0]).astype(BF16)
    head.past(1)
    _wait_all(wq_v, sem_w.at[s_wq])
    row = lax.broadcasted_iota(jnp.int32, (8, PAIR), 0)
    col = lax.broadcasted_iota(jnp.int32, (8, PAIR), 1)
    own = jnp.logical_or(jnp.logical_and(row == 0, col < DH), jnp.logical_and(row == 1, col >= DH))
    for p in range(NPAIR):
        q_s[p] = jnp.where(own, _dot(h, wq_v[:, p * PAIR:(p + 1) * PAIR]), 0.0)
        head.more(PACE)
    head.rest()
    _wait_all(wo_v.at[pl.ds(0, wo_split)], sem_w.at[s_wo])
    att_s[...] = jnp.zeros(att_s.shape, F32)

    def attend(p, slot, stream, step):
        _wait_all(kbuf.at[slot], sem_kv.at[0, slot])
        q = q_s[p].astype(BF16)
        per = nc // QK_STEPS
        for i in range(QK_STEPS):
            for c in range(i * per, (i + 1) * per):
                s_s[:, c * LANE:(c + 1) * LANE] = _dot(q, kbuf[slot, c]) * DH ** -0.5
            stream.more(step)
        s = s_s[...]
        e = jnp.exp(s - jnp.max(s, axis=-1, keepdims=True))
        denom = jnp.sum(e, axis=-1, keepdims=True)
        s_s[...] = e
        stream.more(step)
        _wait_all(vbuf.at[slot], sem_kv.at[1, slot])
        acc = jnp.zeros((8, PAIR), F32)
        per = nc // PV_STEPS
        for i in range(PV_STEPS):
            for c in range(i * per, (i + 1) * per):
                acc += lax.dot_general(s_s[:, c * LANE:(c + 1) * LANE].astype(BF16), vbuf[slot, c],
                                       (((1,), (1,)), ((), ())), preferred_element_type=F32)
            stream.more(step)
        return jnp.where(own, acc / denom, 0.0).astype(BF16)

    def project(p, o):
        r0 = p * PAIR
        if not isinstance(r0, int):
            r0 = pl.multiple_of(r0, PAIR)
        return _dot(o, wo_v[pl.ds(r0, PAIR), :])

    per_pair = 2 * nc * (PAIR // KV_ROWS)

    def body(p, carry):
        stream = _Stream([kv_copies(p + 1, (p + 1) % NSLOT)[LOOP_LOOK:],
                          kv_copies(p + 2, (p + 2) % NSLOT)[:LOOP_LOOK]])
        o = attend(p, p % NSLOT, stream, per_pair // (QK_STEPS + PV_STEPS + 2) // 2 * 2)
        att_s[...] += project(p, o)
        stream.rest()
        return carry

    lax.fori_loop(0, NPAIR - 2, body, 0)

    w1_cols = [(i * F // W1_PARTS, (i + 1) * F // W1_PARTS) for i in range(W1_PARTS)]
    w2_rows, r = [], 0
    for n in W2_ROWS:
        w2_rows.append(((r, r + n), (F // 2 + r, F // 2 + r + n)))
        r += n
    tail = _Stream(
        [kv_copies(NPAIR - 1, (NPAIR - 1) % NSLOT)[LOOP_LOOK:],
         _copies2(wo_hbm, wo_v, sem_w.at[s_wo_tail], (16, D), 1, rows=(wo_split, H * DH))]
        + [_copies2(w1_hbm, w1_v, sem_w.at[s_w1 + i], (16, F // W1_PARTS), 10, cols=cols)
           for i, cols in enumerate(w1_cols)]
        + [_zip2(_copies(w2_hbm, w2_v, sem_w.at[s_w2 + 2 * i], (8, D), 1, rows=ra),
                 _copies(w2_hbm, w2_v, sem_w.at[s_w2 + 2 * i + 1], (8, D), 1, rows=rb))
           for i, (ra, rb) in enumerate(w2_rows)],
        fence)
    o14 = attend(NPAIR - 2, (NPAIR - 2) % NSLOT, tail, PACE)
    tail.past(0)
    o15 = attend(NPAIR - 1, (NPAIR - 1) % NSLOT, tail, PACE)
    tail.past(1)
    _wait_all(wo_v.at[pl.ds(wo_split, H * DH - wo_split)], sem_w.at[s_wo_tail])
    att = att_s[...] + project(NPAIR - 2, o14) + project(NPAIR - 1, o15)
    tail.more(PACE)

    att = jnp.broadcast_to(jnp.sum(att, axis=0, keepdims=True), (8, D))
    x1 = x0 + mod_s[2] * att
    h2 = (_layernorm(x1) * (1.0 + mod_s[4]) + mod_s[3]).astype(BF16)
    tail.more(PACE)
    b1 = b1_v[...].astype(F32)
    acts = []
    for i, (c0, c1) in enumerate(w1_cols):
        tail.past(2 + i)
        _wait_all(w1_v.at[:, pl.ds(c0, c1 - c0)], sem_w.at[s_w1 + i])
        bias = jnp.concatenate(
            [jnp.broadcast_to(b1[t:t + 1, :], (8, LANE)) for t in range(c0 // LANE, c1 // LANE)], axis=1)
        acts.append(_mish(_dot(h2, w1_v[:, c0:c1]) + bias).astype(BF16))
        tail.more(PACE)
    act = jnp.concatenate(acts, axis=1)
    y = jnp.zeros((8, D), F32)
    for i, t in W2_ORDER:
        ra, rb = w2_rows[i][t]
        tail.past(2 + W1_PARTS + i)
        _wait_all(w2_v.at[pl.ds(ra, rb - ra)], sem_w.at[s_w2 + 2 * i + t])
        y += _dot(act[:, ra:rb], w2_v[ra:rb, :])
    o_ref[...] = (x1 + mod_s[5] * y)[0:1].astype(o_ref.dtype)


@jax.jit
def pallas_adaLN_cond__sliding_block_cached__dense_activation_mish__decode_kernel(
    A_x: jax.Array,
    A_k_cache: jax.Array,
    A_v_cache: jax.Array,
    A_wq: jax.Array,
    A_wo: jax.Array,
    B_x: jax.Array,
    B_w1: jax.Array,
    B_b1: jax.Array,
    B_w2: jax.Array,
    c: jax.Array,
    w_mod: jax.Array,
):
    del B_x
    sk = A_k_cache.shape[2]
    window = min(4096, max(256, sk // 4))
    kt = jnp.swapaxes(A_k_cache, 2, 3).reshape(H * DH, sk)
    vt = jnp.swapaxes(A_v_cache, 2, 3).reshape(H * DH, sk)
    hbm = pl.BlockSpec(memory_space=pltpu.HBM)
    out = pl.pallas_call(
        functools.partial(_kernel, window=window),
        out_shape=jax.ShapeDtypeStruct((1, D), A_x.dtype),
        in_specs=[hbm] * 10,
        out_specs=pl.BlockSpec(memory_space=pltpu.VMEM),
        scratch_shapes=[
            pltpu.VMEM((1, D), BF16),
            pltpu.VMEM((1, D), BF16),
            pltpu.VMEM((F // LANE, LANE), BF16),
            pltpu.VMEM((D, 6 * D), BF16),
            pltpu.VMEM((D, H * DH), BF16),
            pltpu.VMEM((H * DH, D), BF16),
            pltpu.VMEM((D, F), BF16),
            pltpu.VMEM((F, D), BF16),
            pltpu.VMEM((NSLOT, window // LANE, PAIR, LANE), BF16),
            pltpu.VMEM((NSLOT, window // LANE, PAIR, LANE), BF16),
            pltpu.VMEM((NPAIR, 8, PAIR), F32),
            pltpu.VMEM((8, window), F32),
            pltpu.VMEM((8, D), F32),
            pltpu.VMEM((6, 8, D), F32),
            pltpu.SemaphoreType.DMA((7 + W1_PARTS + 2 * len(W2_ROWS),)),
            pltpu.SemaphoreType.DMA((2, NSLOT)),
            pltpu.SemaphoreType.REGULAR,
        ],
        compiler_params=pltpu.CompilerParams(
            vmem_limit_bytes=64 * 2**20,
            disable_bounds_checks=True,
            disable_semaphore_checks=True,
        ),
        name="adaln_attn_mlp_decode",
    )(A_x.reshape(1, D), kt, vt, A_wq, A_wo, B_w1, B_b1.reshape(F // LANE, LANE), B_w2, c, w_mod)
    return out.reshape(A_x.shape)
```

```python
import functools

import jax
import jax.numpy as jnp
from jax import lax
import jax.experimental.pallas as pl
import jax.experimental.pallas.tpu as pltpu

D = 640
H = 32
DH = 192
F = 1536
PAIR = 2 * DH
NPAIR = H // 2
LANE = 128
F32 = jnp.float32
BF16 = jnp.bfloat16

KV_ROWS = 96
NSLOT = 3
LOOK = 80
LOOP_LOOK = 128
PACE = 10
QK_STEPS = 4
PV_STEPS = 4
W1_PARTS = 2
W2_ROWS = (384, 256, 128)
W2_ORDER = ((0, 0), (0, 1), (1, 0), (2, 0), (1, 1), (2, 1))


def _layernorm(x, eps=1e-5):
    m = jnp.mean(x, axis=-1, keepdims=True)
    d = x - m
    v = jnp.mean(d * d, axis=-1, keepdims=True)
    return d / jnp.sqrt(v + eps)


def _mish(u):
    softplus = jnp.log1p(jnp.exp(-jnp.abs(u))) + jnp.where(u > 0, u, 0.0)
    return u * jnp.tanh(softplus)


def _dot(a, b):
    return jnp.dot(a, b, preferred_element_type=F32)


def _zip2(a, b):
    n = min(len(a), len(b))
    out = [x for p in zip(a[:n], b[:n]) for x in p]
    rest = a[n:] + b[n:]
    h = len(rest) // 2
    return out + [x for p in zip(rest[:h], rest[h:2 * h]) for x in p] + rest[2 * h:]


class _Stream:
    def __init__(self, parts, fence=None):
        self.copies = [cp for part in parts for cp in part]
        self.ends = []
        n = 0
        for part in parts:
            n += len(part)
            self.ends.append(n)
        self.fence = fence
        self.pos = 0

    def upto(self, n):
        n = min(n, len(self.copies))
        while self.pos < n:
            if self.fence is not None and self.pos in self.ends:
                self.fence()
            self.copies[self.pos]().start(priority=self.pos % 2)
            self.pos += 1

    def more(self, k):
        self.upto(self.pos + k)

    def past(self, part):
        self.upto(self.ends[part] + LOOK)

    def rest(self):
        self.upto(len(self.copies))


def _copies(src, dst, sem, shape, jump, rows=None, cols=None):
    r0, r1 = rows or (0, src.shape[0])
    c0, c1 = cols or (0, src.shape[1])
    rr, cc = shape
    assert (r1 - r0) % rr == 0 and (c1 - c0) % cc == 0
    idx = [(r, c) for c in range(c0, c1, cc) for r in range(r0, r1, rr)]
    idx = [idx[i] for o in range(jump) for i in range(o, len(idx), jump)]
    return [functools.partial(pltpu.make_async_copy, src.at[pl.ds(r, rr), pl.ds(c, cc)],
                              dst.at[pl.ds(r, rr), pl.ds(c, cc)], sem) for r, c in idx]


def _copies2(src, dst, sem, shape, jump, rows=None, cols=None):
    r0, r1 = rows or (0, src.shape[0])
    mid = (r0 + r1) // 2
    return _zip2(_copies(src, dst, sem, shape, jump, (r0, mid), cols),
                 _copies(src, dst, sem, shape, jump, (mid, r1), cols))


def _wait_all(buf, sem):
    pltpu.make_async_copy(buf, buf, sem).wait()


def _kernel(x_hbm, k_hbm, v_hbm, wq_hbm, wo_hbm, w1_hbm, b1_hbm, w2_hbm, c_hbm, wmod_hbm, o_ref,
            x_v, c_v, b1_v, wmod_v, wq_v, wo_v, w1_v, w2_v, kbuf, vbuf, q_s, s_s, att_s, mod_s,
            sem_w, sem_kv, sem_fence, *, window):
    sk = k_hbm.shape[1]
    nc = window // LANE

    def kv_copies(p, slot):
        out = []
        for r in range(0, PAIR, KV_ROWS):
            row = p * PAIR + r
            if not isinstance(row, int):
                row = pl.multiple_of(row, 8)
            for c in range(nc):
                for j, (src, dst) in enumerate(((k_hbm, kbuf), (v_hbm, vbuf))):
                    out.append(functools.partial(
                        pltpu.make_async_copy,
                        src.at[pl.ds(row, KV_ROWS), pl.ds(sk - window + c * LANE, LANE)],
                        dst.at[slot, c, pl.ds(r, KV_ROWS), :], sem_kv.at[j, slot]))
        return out

    def fence():
        pl.semaphore_signal(sem_fence, 1)
        pl.semaphore_wait(sem_fence, 1)

    s_c, s_x, s_b1, s_wmod, s_wq, s_wo, s_wo_tail, s_w1 = range(8)
    s_w2 = s_w1 + W1_PARTS
    small = [functools.partial(pltpu.make_async_copy, s, d, sem_w.at[i])
             for i, s, d in ((s_c, c_hbm, c_v), (s_x, x_hbm, x_v), (s_b1, b1_hbm, b1_v))]
    wo_split = (NPAIR - 2) * PAIR

    head = _Stream([
        _copies2(wmod_hbm, wmod_v, sem_w.at[s_wmod], (8, 1280), 8),
        _zip2(_copies(wq_hbm, wq_v, sem_w.at[s_wq], (8, 1536), 8),
              _copies(wo_hbm, wo_v, sem_w.at[s_wo], (24, D), 48, rows=(0, wo_split))),
        kv_copies(0, 0),
        kv_copies(1, 1)[:LOOP_LOOK],
    ], fence)
    head.upto(2)
    for cp in small:
        cp().start()
    head.past(0)
    for cp in small:
        cp().wait()
    _wait_all(wmod_v, sem_w.at[s_wmod])
    cf = c_v[...].astype(F32)
    silu_c = jnp.broadcast_to(cf * jax.nn.sigmoid(cf), (8, D)).astype(BF16)
    for i in range(6):
        mod_s[i] = _dot(silu_c, wmod_v[:, i * D:(i + 1) * D])
        head.more(PACE)
    x0 = jnp.broadcast_to(x_v[...].astype(F32), (8, D))
    h = (_layernorm(x0) * (1.0 + mod_s[1]) + mod_s[0]).astype(BF16)
    head.past(1)
    _wait_all(wq_v, sem_w.at[s_wq])
    row = lax.broadcasted_iota(jnp.int32, (8, PAIR), 0)
    col = lax.broadcasted_iota(jnp.int32, (8, PAIR), 1)
    own = jnp.logical_or(jnp.logical_and(row == 0, col < DH), jnp.logical_and(row == 1, col >= DH))
    for p in range(NPAIR):
        q_s[p] = jnp.where(own, _dot(h, wq_v[:, p * PAIR:(p + 1) * PAIR]), 0.0)
        head.more(PACE)
    head.rest()
    _wait_all(wo_v.at[pl.ds(0, wo_split)], sem_w.at[s_wo])
    att_s[...] = jnp.zeros(att_s.shape, F32)

    def attend(p, slot, stream, step):
        _wait_all(kbuf.at[slot], sem_kv.at[0, slot])
        q = q_s[p].astype(BF16)
        per = nc // QK_STEPS
        for i in range(QK_STEPS):
            for c in range(i * per, (i + 1) * per):
                s_s[:, c * LANE:(c + 1) * LANE] = _dot(q, kbuf[slot, c]) * DH ** -0.5
            stream.more(step)
        s = s_s[...]
        e = jnp.exp(s - jnp.max(s, axis=-1, keepdims=True))
        denom = jnp.sum(e, axis=-1, keepdims=True)
        s_s[...] = e
        stream.more(step)
        _wait_all(vbuf.at[slot], sem_kv.at[1, slot])
        acc = jnp.zeros((8, PAIR), F32)
        per = nc // PV_STEPS
        for i in range(PV_STEPS):
            for c in range(i * per, (i + 1) * per):
                acc += lax.dot_general(s_s[:, c * LANE:(c + 1) * LANE].astype(BF16), vbuf[slot, c],
                                       (((1,), (1,)), ((), ())), preferred_element_type=F32)
            stream.more(step)
        return jnp.where(own, acc / denom, 0.0).astype(BF16)

    def project(p, o):
        r0 = p * PAIR
        if not isinstance(r0, int):
            r0 = pl.multiple_of(r0, PAIR)
        return _dot(o, wo_v[pl.ds(r0, PAIR), :])

    per_pair = 2 * nc * (PAIR // KV_ROWS)

    def body(p, carry):
        stream = _Stream([kv_copies(p + 1, (p + 1) % NSLOT)[LOOP_LOOK:],
                          kv_copies(p + 2, (p + 2) % NSLOT)[:LOOP_LOOK]])
        o = attend(p, p % NSLOT, stream, per_pair // (QK_STEPS + PV_STEPS + 2) // 2 * 2)
        att_s[...] += project(p, o)
        stream.rest()
        return carry

    lax.fori_loop(0, NPAIR - 2, body, 0)

    w1_cols = [(i * F // W1_PARTS, (i + 1) * F // W1_PARTS) for i in range(W1_PARTS)]
    w2_rows, r = [], 0
    for n in W2_ROWS:
        w2_rows.append(((r, r + n), (F // 2 + r, F // 2 + r + n)))
        r += n
    tail = _Stream(
        [kv_copies(NPAIR - 1, (NPAIR - 1) % NSLOT)[LOOP_LOOK:],
         _copies2(wo_hbm, wo_v, sem_w.at[s_wo_tail], (16, D), 1, rows=(wo_split, H * DH))]
        + [_copies2(w1_hbm, w1_v, sem_w.at[s_w1 + i], (16, F // W1_PARTS), 10, cols=cols)
           for i, cols in enumerate(w1_cols)]
        + [_zip2(_copies(w2_hbm, w2_v, sem_w.at[s_w2 + 2 * i], (8, D), 1, rows=ra),
                 _copies(w2_hbm, w2_v, sem_w.at[s_w2 + 2 * i + 1], (8, D), 1, rows=rb))
           for i, (ra, rb) in enumerate(w2_rows)],
        fence)
    o14 = attend(NPAIR - 2, (NPAIR - 2) % NSLOT, tail, PACE)
    tail.past(0)
    o15 = attend(NPAIR - 1, (NPAIR - 1) % NSLOT, tail, PACE)
    tail.past(1)
    _wait_all(wo_v.at[pl.ds(wo_split, H * DH - wo_split)], sem_w.at[s_wo_tail])
    att = att_s[...] + project(NPAIR - 2, o14) + project(NPAIR - 1, o15)
    tail.more(PACE)

    att = jnp.broadcast_to(jnp.sum(att, axis=0, keepdims=True), (8, D))
    x1 = x0 + mod_s[2] * att
    h2 = (_layernorm(x1) * (1.0 + mod_s[4]) + mod_s[3]).astype(BF16)
    tail.more(PACE)
    b1 = b1_v[...].astype(F32)
    acts = []
    for i, (c0, c1) in enumerate(w1_cols):
        tail.past(2 + i)
        _wait_all(w1_v.at[:, pl.ds(c0, c1 - c0)], sem_w.at[s_w1 + i])
        bias = jnp.concatenate(
            [jnp.broadcast_to(b1[t:t + 1, :], (8, LANE)) for t in range(c0 // LANE, c1 // LANE)], axis=1)
        acts.append(_mish(_dot(h2, w1_v[:, c0:c1]) + bias).astype(BF16))
        tail.more(PACE)
    act = jnp.concatenate(acts, axis=1)
    y = jnp.zeros((8, D), F32)
    for i, t in W2_ORDER:
        ra, rb = w2_rows[i][t]
        tail.past(2 + W1_PARTS + i)
        _wait_all(w2_v.at[pl.ds(ra, rb - ra)], sem_w.at[s_w2 + 2 * i + t])
        y += _dot(act[:, ra:rb], w2_v[ra:rb, :])
    o_ref[...] = (x1 + mod_s[5] * y)[0:1].astype(o_ref.dtype)


@jax.jit
def pallas_adaLN_cond__sliding_block_cached__dense_activation_mish__decode_kernel(
    A_x: jax.Array,
    A_k_cache: jax.Array,
    A_v_cache: jax.Array,
    A_wq: jax.Array,
    A_wo: jax.Array,
    B_x: jax.Array,
    B_w1: jax.Array,
    B_b1: jax.Array,
    B_w2: jax.Array,
    c: jax.Array,
    w_mod: jax.Array,
):
    del B_x
    sk = A_k_cache.shape[2]
    window = min(4096, max(256, sk // 4))
    kt = jnp.swapaxes(A_k_cache, 2, 3).reshape(H * DH, sk)
    vt = jnp.swapaxes(A_v_cache, 2, 3).reshape(H * DH, sk)
    hbm = pl.BlockSpec(memory_space=pltpu.HBM)
    out = pl.pallas_call(
        functools.partial(_kernel, window=window),
        out_shape=jax.ShapeDtypeStruct((1, D), A_x.dtype),
        in_specs=[hbm] * 10,
        out_specs=pl.BlockSpec(memory_space=pltpu.VMEM),
        scratch_shapes=[
            pltpu.VMEM((1, D), BF16),
            pltpu.VMEM((1, D), BF16),
            pltpu.VMEM((F // LANE, LANE), BF16),
            pltpu.VMEM((D, 6 * D), BF16),
            pltpu.VMEM((D, H * DH), BF16),
            pltpu.VMEM((H * DH, D), BF16),
            pltpu.VMEM((D, F), BF16),
            pltpu.VMEM((F, D), BF16),
            pltpu.VMEM((NSLOT, window // LANE, PAIR, LANE), BF16),
            pltpu.VMEM((NSLOT, window // LANE, PAIR, LANE), BF16),
            pltpu.VMEM((NPAIR, 8, PAIR), F32),
            pltpu.VMEM((8, window), F32),
            pltpu.VMEM((8, D), F32),
            pltpu.VMEM((6, 8, D), F32),
            pltpu.SemaphoreType.DMA((7 + W1_PARTS + 2 * len(W2_ROWS),)),
            pltpu.SemaphoreType.DMA((2, NSLOT)),
            pltpu.SemaphoreType.REGULAR,
        ],
        compiler_params=pltpu.CompilerParams(
            vmem_limit_bytes=64 * 2**20,
            disable_semaphore_checks=True,
        ),
        name="adaln_attn_mlp_decode",
    )(A_x.reshape(1, D), kt, vt, A_wq, A_wo, B_w1, B_b1.reshape(F // LANE, LANE), B_w2, c, w_mod)
    return out.reshape(A_x.shape)
```

```python
import functools

import jax
import jax.numpy as jnp
from jax import lax
import jax.experimental.pallas as pl
import jax.experimental.pallas.tpu as pltpu

D = 640
H = 32
DH = 192
F = 1536
PAIR = 2 * DH
NPAIR = H // 2
LANE = 128
F32 = jnp.float32
BF16 = jnp.bfloat16

KV_ROWS = 96
NSLOT = 3
LOOK = 80
MLP_LOOK = 120
LOOP_LOOK = 128
PACE = 10
QK_STEPS = 4
PV_STEPS = 4
W1_PARTS = 2
W2_ROWS = (384, 256, 128)
W2_ORDER = ((0, 0), (0, 1), (1, 0), (2, 0), (1, 1), (2, 1))


def _layernorm(x, eps=1e-5):
    m = jnp.mean(x, axis=-1, keepdims=True)
    d = x - m
    v = jnp.mean(d * d, axis=-1, keepdims=True)
    return d / jnp.sqrt(v + eps)


def _mish(u):
    softplus = jnp.log1p(jnp.exp(-jnp.abs(u))) + jnp.where(u > 0, u, 0.0)
    return u * jnp.tanh(softplus)


def _dot(a, b):
    return jnp.dot(a, b, preferred_element_type=F32)


def _zip2(a, b):
    n = min(len(a), len(b))
    out = [x for p in zip(a[:n], b[:n]) for x in p]
    rest = a[n:] + b[n:]
    h = len(rest) // 2
    return out + [x for p in zip(rest[:h], rest[h:2 * h]) for x in p] + rest[2 * h:]


class _Stream:
    def __init__(self, parts, fence=None):
        self.copies = [cp for part in parts for cp in part]
        self.ends = []
        n = 0
        for part in parts:
            n += len(part)
            self.ends.append(n)
        self.fence = fence
        self.pos = 0

    def upto(self, n):
        n = min(n, len(self.copies))
        while self.pos < n:
            if self.fence is not None and self.pos in self.ends:
                self.fence()
            self.copies[self.pos]().start(priority=self.pos % 2)
            self.pos += 1

    def more(self, k):
        self.upto(self.pos + k)

    def past(self, part, look=LOOK):
        self.upto(self.ends[part] + look)

    def rest(self):
        self.upto(len(self.copies))


def _copies(src, dst, sem, shape, jump, rows=None, cols=None):
    r0, r1 = rows or (0, src.shape[0])
    c0, c1 = cols or (0, src.shape[1])
    rr, cc = shape
    assert (r1 - r0) % rr == 0 and (c1 - c0) % cc == 0
    idx = [(r, c) for c in range(c0, c1, cc) for r in range(r0, r1, rr)]
    idx = [idx[i] for o in range(jump) for i in range(o, len(idx), jump)]
    return [functools.partial(pltpu.make_async_copy, src.at[pl.ds(r, rr), pl.ds(c, cc)],
                              dst.at[pl.ds(r, rr), pl.ds(c, cc)], sem) for r, c in idx]


def _copies2(src, dst, sem, shape, jump, rows=None, cols=None):
    r0, r1 = rows or (0, src.shape[0])
    mid = (r0 + r1) // 2
    return _zip2(_copies(src, dst, sem, shape, jump, (r0, mid), cols),
                 _copies(src, dst, sem, shape, jump, (mid, r1), cols))


def _wait_all(buf, sem):
    pltpu.make_async_copy(buf, buf, sem).wait()


def _kernel(x_hbm, k_hbm, v_hbm, wq_hbm, wo_hbm, w1_hbm, b1_hbm, w2_hbm, c_hbm, wmod_hbm, o_ref,
            x_v, c_v, b1_v, wmod_v, wq_v, wo_v, w1_v, w2_v, kbuf, vbuf, q_s, s_s, att_s, mod_s,
            sem_w, sem_kv, sem_fence, *, window):
    sk = k_hbm.shape[1]
    nc = window // LANE

    def kv_copies(p, slot):
        out = []
        for r in range(0, PAIR, KV_ROWS):
            row = p * PAIR + r
            if not isinstance(row, int):
                row = pl.multiple_of(row, 8)
            for c in range(nc):
                for j, (src, dst) in enumerate(((k_hbm, kbuf), (v_hbm, vbuf))):
                    out.append(functools.partial(
                        pltpu.make_async_copy,
                        src.at[pl.ds(row, KV_ROWS), pl.ds(sk - window + c * LANE, LANE)],
                        dst.at[slot, c, pl.ds(r, KV_ROWS), :], sem_kv.at[j, slot]))
        return out

    def fence():
        pl.semaphore_signal(sem_fence, 1)
        pl.semaphore_wait(sem_fence, 1)

    s_c, s_x, s_b1, s_wmod, s_wq, s_wo, s_wo_tail, s_w1 = range(8)
    s_w2 = s_w1 + W1_PARTS
    small = [functools.partial(pltpu.make_async_copy, s, d, sem_w.at[i])
             for i, s, d in ((s_c, c_hbm, c_v), (s_x, x_hbm, x_v), (s_b1, b1_hbm, b1_v))]
    wo_split = (NPAIR - 2) * PAIR

    head = _Stream([
        _copies2(wmod_hbm, wmod_v, sem_w.at[s_wmod], (8, 1280), 8),
        _zip2(_copies(wq_hbm, wq_v, sem_w.at[s_wq], (8, 2048), 16),
              _copies(wo_hbm, wo_v, sem_w.at[s_wo], (24, D), 48, rows=(0, wo_split))),
        kv_copies(0, 0),
        kv_copies(1, 1)[:LOOP_LOOK],
    ], fence)
    head.upto(2)
    for cp in small:
        cp().start()
    head.past(0)
    for cp in small:
        cp().wait()
    _wait_all(wmod_v, sem_w.at[s_wmod])
    cf = c_v[...].astype(F32)
    silu_c = jnp.broadcast_to(cf * jax.nn.sigmoid(cf), (8, D)).astype(BF16)
    for i in range(6):
        mod_s[i] = _dot(silu_c, wmod_v[:, i * D:(i + 1) * D])
        head.more(PACE)
    x0 = jnp.broadcast_to(x_v[...].astype(F32), (8, D))
    h = (_layernorm(x0) * (1.0 + mod_s[1]) + mod_s[0]).astype(BF16)
    head.past(1)
    _wait_all(wq_v, sem_w.at[s_wq])
    row = lax.broadcasted_iota(jnp.int32, (8, PAIR), 0)
    col = lax.broadcasted_iota(jnp.int32, (8, PAIR), 1)
    own = jnp.logical_or(jnp.logical_and(row == 0, col < DH), jnp.logical_and(row == 1, col >= DH))
    for p in range(NPAIR):
        q_s[p] = jnp.where(own, _dot(h, wq_v[:, p * PAIR:(p + 1) * PAIR]), 0.0)
        head.more(PACE)
    head.rest()
    _wait_all(wo_v.at[pl.ds(0, wo_split)], sem_w.at[s_wo])
    att_s[...] = jnp.zeros(att_s.shape, F32)

    def attend(p, slot, stream, step):
        _wait_all(kbuf.at[slot], sem_kv.at[0, slot])
        q = q_s[p].astype(BF16)
        per = nc // QK_STEPS
        for i in range(QK_STEPS):
            for c in range(i * per, (i + 1) * per):
                s_s[:, c * LANE:(c + 1) * LANE] = _dot(q, kbuf[slot, c]) * DH ** -0.5
            stream.more(step)
        s = s_s[...]
        e = jnp.exp(s - jnp.max(s, axis=-1, keepdims=True))
        denom = jnp.sum(e, axis=-1, keepdims=True)
        s_s[...] = e
        stream.more(step)
        _wait_all(vbuf.at[slot], sem_kv.at[1, slot])
        acc = jnp.zeros((8, PAIR), F32)
        per = nc // PV_STEPS
        for i in range(PV_STEPS):
            for c in range(i * per, (i + 1) * per):
                acc += lax.dot_general(s_s[:, c * LANE:(c + 1) * LANE].astype(BF16), vbuf[slot, c],
                                       (((1,), (1,)), ((), ())), preferred_element_type=F32)
            stream.more(step)
        return jnp.where(own, acc / denom, 0.0).astype(BF16)

    def project(p, o):
        r0 = p * PAIR
        if not isinstance(r0, int):
            r0 = pl.multiple_of(r0, PAIR)
        return _dot(o, wo_v[pl.ds(r0, PAIR), :])

    per_pair = 2 * nc * (PAIR // KV_ROWS)

    def body(p, carry):
        stream = _Stream([kv_copies(p + 1, (p + 1) % NSLOT)[LOOP_LOOK:],
                          kv_copies(p + 2, (p + 2) % NSLOT)[:LOOP_LOOK]])
        o = attend(p, p % NSLOT, stream, per_pair // (QK_STEPS + PV_STEPS + 2) // 2 * 2)
        att_s[...] += project(p, o)
        stream.rest()
        return carry

    lax.fori_loop(0, NPAIR - 2, body, 0)

    w1_cols = [(i * F // W1_PARTS, (i + 1) * F // W1_PARTS) for i in range(W1_PARTS)]
    w2_rows, r = [], 0
    for n in W2_ROWS:
        w2_rows.append(((r, r + n), (F // 2 + r, F // 2 + r + n)))
        r += n
    tail = _Stream(
        [kv_copies(NPAIR - 1, (NPAIR - 1) % NSLOT)[LOOP_LOOK:],
         _copies2(wo_hbm, wo_v, sem_w.at[s_wo_tail], (16, D), 1, rows=(wo_split, H * DH))]
        + [_copies2(w1_hbm, w1_v, sem_w.at[s_w1 + i], (16, F // W1_PARTS), 10, cols=cols)
           for i, cols in enumerate(w1_cols)]
        + [_zip2(_copies(w2_hbm, w2_v, sem_w.at[s_w2 + 2 * i], (8, D), 1, rows=ra),
                 _copies(w2_hbm, w2_v, sem_w.at[s_w2 + 2 * i + 1], (8, D), 1, rows=rb))
           for i, (ra, rb) in enumerate(w2_rows)],
        fence)
    o14 = attend(NPAIR - 2, (NPAIR - 2) % NSLOT, tail, PACE)
    tail.past(0)
    o15 = attend(NPAIR - 1, (NPAIR - 1) % NSLOT, tail, PACE)
    tail.past(1)
    _wait_all(wo_v.at[pl.ds(wo_split, H * DH - wo_split)], sem_w.at[s_wo_tail])
    att = att_s[...] + project(NPAIR - 2, o14) + project(NPAIR - 1, o15)
    tail.more(PACE)

    att = jnp.broadcast_to(jnp.sum(att, axis=0, keepdims=True), (8, D))
    x1 = x0 + mod_s[2] * att
    h2 = (_layernorm(x1) * (1.0 + mod_s[4]) + mod_s[3]).astype(BF16)
    tail.more(PACE)
    b1 = b1_v[...].astype(F32)
    acts = []
    for i, (c0, c1) in enumerate(w1_cols):
        tail.past(2 + i, MLP_LOOK)
        _wait_all(w1_v.at[:, pl.ds(c0, c1 - c0)], sem_w.at[s_w1 + i])
        bias = jnp.concatenate(
            [jnp.broadcast_to(b1[t:t + 1, :], (8, LANE)) for t in range(c0 // LANE, c1 // LANE)], axis=1)
        acts.append(_mish(_dot(h2, w1_v[:, c0:c1]) + bias).astype(BF16))
        tail.more(PACE)
    act = jnp.concatenate(acts, axis=1)
    y = jnp.zeros((8, D), F32)
    for i, t in W2_ORDER:
        ra, rb = w2_rows[i][t]
        tail.past(2 + W1_PARTS + i, MLP_LOOK)
        _wait_all(w2_v.at[pl.ds(ra, rb - ra)], sem_w.at[s_w2 + 2 * i + t])
        y += _dot(act[:, ra:rb], w2_v[ra:rb, :])
    o_ref[...] = (x1 + mod_s[5] * y)[0:1].astype(o_ref.dtype)


@jax.jit
def pallas_adaLN_cond__sliding_block_cached__dense_activation_mish__decode_kernel(
    A_x: jax.Array,
    A_k_cache: jax.Array,
    A_v_cache: jax.Array,
    A_wq: jax.Array,
    A_wo: jax.Array,
    B_x: jax.Array,
    B_w1: jax.Array,
    B_b1: jax.Array,
    B_w2: jax.Array,
    c: jax.Array,
    w_mod: jax.Array,
):
    del B_x
    sk = A_k_cache.shape[2]
    window = min(4096, max(256, sk // 4))
    kt = jnp.swapaxes(A_k_cache, 2, 3).reshape(H * DH, sk)
    vt = jnp.swapaxes(A_v_cache, 2, 3).reshape(H * DH, sk)
    hbm = pl.BlockSpec(memory_space=pltpu.HBM)
    out = pl.pallas_call(
        functools.partial(_kernel, window=window),
        out_shape=jax.ShapeDtypeStruct((1, D), A_x.dtype),
        in_specs=[hbm] * 10,
        out_specs=pl.BlockSpec(memory_space=pltpu.VMEM),
        scratch_shapes=[
            pltpu.VMEM((1, D), BF16),
            pltpu.VMEM((1, D), BF16),
            pltpu.VMEM((F // LANE, LANE), BF16),
            pltpu.VMEM((D, 6 * D), BF16),
            pltpu.VMEM((D, H * DH), BF16),
            pltpu.VMEM((H * DH, D), BF16),
            pltpu.VMEM((D, F), BF16),
            pltpu.VMEM((F, D), BF16),
            pltpu.VMEM((NSLOT, window // LANE, PAIR, LANE), BF16),
            pltpu.VMEM((NSLOT, window // LANE, PAIR, LANE), BF16),
            pltpu.VMEM((NPAIR, 8, PAIR), F32),
            pltpu.VMEM((8, window), F32),
            pltpu.VMEM((8, D), F32),
            pltpu.VMEM((6, 8, D), F32),
            pltpu.SemaphoreType.DMA((7 + W1_PARTS + 2 * len(W2_ROWS),)),
            pltpu.SemaphoreType.DMA((2, NSLOT)),
            pltpu.SemaphoreType.REGULAR,
        ],
        compiler_params=pltpu.CompilerParams(
            vmem_limit_bytes=64 * 2**20,
            disable_semaphore_checks=True,
        ),
        name="adaln_attn_mlp_decode",
    )(A_x.reshape(1, D), kt, vt, A_wq, A_wo, B_w1, B_b1.reshape(F // LANE, LANE), B_w2, c, w_mod)
    return out.reshape(A_x.shape)
```
